```python
import jax
import jax.numpy as jnp

def _softmax(x, axis=-1):
    return jax.nn.softmax(x, axis=axis)
def _gelu(x):
    return jax.nn.gelu(x, approximate=True)
def _silu(x):
    return jax.nn.silu(x)
def _sigmoid(x):
    return jax.nn.sigmoid(x)
def _layernorm(x, axis=-1, eps=1e-5):
    m = jnp.mean(x, axis=axis, keepdims=True)
    v = jnp.var(x, axis=axis, keepdims=True)
    return (x - m) / jnp.sqrt(v + eps)
def _scatter_add(tgt, idx, src, axis=0):
    return tgt.at[idx].add(src)
def _segment_sum(src, seg, n):
    return jax.ops.segment_sum(src, seg, n)
class _Rng:
    def __init__(self, key):
        self._k = key
    def _next(self):
        self._k, sub = jax.random.split(self._k)
        return sub
    def normal(self, shape):
        return jax.random.normal(self._next(), shape, dtype=jnp.bfloat16)
    def randint(self, lo, hi, shape):
        return jax.random.randint(self._next(), shape, lo, hi, dtype=jnp.int32)
    def uniform(self, shape, lo=0.0, hi=1.0):
        return jax.random.uniform(self._next(), shape, jnp.bfloat16, lo, hi)
    def permutation(self, n):
        return jax.random.permutation(self._next(), n)


kernel_name = 'recurrent_scan__linear_kernel_hedgehog__dense_activation_relu__prompt'

def _fwd_setup_inputs():
    _rng = _Rng(jax.random.key(int.from_bytes(__import__("os").urandom(4), "little")))
    _w = (lambda a: (lambda t: t.astype(jnp.bfloat16) if jnp.issubdtype(t.dtype, jnp.floating) else t)(jnp.asarray(a)))
    def _A_setup():
        B, S, D, H = 1, 2048, 1024, 32
        Dh = D // H
        return {
            "x": _w((lambda *s: _rng.normal(s) * 0.05)(B, S, D)),
            "wqkv": _w((lambda *s: _rng.normal(s) * 0.05)(D, 3 * D)),
            "w_phi": _w((lambda *s: _rng.normal(s) * 0.05)(H, Dh, Dh) * (Dh ** -0.5)),
            "wo": _w((lambda *s: _rng.normal(s) * 0.05)(D, D)),
        }
    _A_in = _A_setup()

    def _B_setup():
        B, S, D, Dff = 1, 2048, 1024, 3584
        return {
            "x": _w((lambda *s: _rng.normal(s) * 0.05)(B, S, D)),
            "w1": _w((lambda *s: _rng.normal(s) * 0.05)(D, Dff)),
            "w2": _w((lambda *s: _rng.normal(s) * 0.05)(Dff, D)),
        }
    _B_in = _B_setup()

    return {
        "A_x": _A_in["x"],
        "A_wqkv": _A_in["wqkv"],
        "A_w_phi": _A_in["w_phi"],
        "A_wo": _A_in["wo"],
        "B_x": _B_in["x"],
        "B_w1": _B_in["w1"],
        "B_w2": _B_in["w2"],
    }

def _fwd_reference(A_x, A_wqkv, A_w_phi, A_wo, B_x, B_w1, B_w2):
    def _A_ref(x, wqkv, w_phi, wo):
        B, S, D = x.shape
        H = 32; Dh = D // H
        qkv = (lambda x, *d: x.transpose(*d))((x @ wqkv).reshape(B, S, 3, H, Dh), 2, 0, 3, 1, 4)
        q, k, v = qkv[0], qkv[1], qkv[2]
        pq = jnp.einsum("bhsd,hdf->bhsf", q, w_phi)
        pk = jnp.einsum("bhsd,hdf->bhsf", k, w_phi)
        phi_q = jnp.concatenate([_softmax(pq, axis=-1), _softmax(-pq, axis=-1)], axis=-1)
        phi_k = jnp.concatenate([_softmax(pk, axis=-1), _softmax(-pk, axis=-1)], axis=-1)
        kv = jnp.einsum("bhsf,bhsd->bhfd", phi_k, v)
        z  = jnp.einsum("bhsf->bhf", phi_k)
        num = jnp.einsum("bhqf,bhfd->bhqd", phi_q, kv)
        den = jnp.einsum("bhqf,bhf->bhq", phi_q, z)[..., None] + 1e-6
        o = num / den
        return (lambda x, *d: x.transpose(*d))(o, 0, 2, 1, 3).reshape(B, S, D) @ wo

    def _B_ref(x, w1, w2):
        h = jnp.einsum("bsd,df->bsf", x, w1)
        zero = jnp.zeros_like(h)
        h = jnp.maximum(h, zero)
        return jnp.einsum("bsf,fd->bsd", h, w2)

    x = A_x
    xn = _layernorm(x, axis=-1)
    s = _A_ref(xn, A_wqkv, A_w_phi, A_wo)
    g = _silu(_B_ref(xn, B_w1, B_w2))
    return x + s * g


def setup_inputs():
    _inp = _fwd_setup_inputs()
    _gk = jax.random.fold_in(jax.random.key(int.from_bytes(__import__("os").urandom(4), "little")), 2**31 - 1)
    _shapes = [[1, 2048, 1024]]
    _dtypes = ['bfloat16']
    _gks = jax.random.split(_gk, len(_shapes))
    _gs = [jax.random.normal(k, s, dtype=jnp.dtype(d)) * 0.05 for k, s, d in zip(_gks, _shapes, _dtypes)]
    _inp["grad_out"] = _gs[0]
    return _inp

def reference(A_x, A_wqkv, A_w_phi, A_wo, B_w1, B_w2, B_x, grad_out):
    _const = dict(B_x=B_x)
    def _f(*_d):
        return _fwd_reference(**{'A_x': _d[0], 'A_wqkv': _d[1], 'A_w_phi': _d[2], 'A_wo': _d[3], 'B_w1': _d[4], 'B_w2': _d[5], **_const})
    _out, _vjp = jax.vjp(_f, A_x, A_wqkv, A_w_phi, A_wo, B_w1, B_w2)
    _grads = _vjp(grad_out)
    _out0 = jnp.asarray(_out)
    return (_out0, *[jnp.asarray(_g) for _g in _grads])
```

```python
import jax
import jax.numpy as jnp
from jax import lax
import jax.experimental.pallas as pl
import jax.experimental.pallas.tpu as pltpu

S, D, H, F = 2048, 1024, 32, 3584
DH = D // H
T = 512
NT = S // T
FC = 512
NC = F // FC
G = D // 128
EXT = 16
BF, F32 = jnp.bfloat16, jnp.float32


def _nn(a, b):
    return lax.dot_general(a, b, (((1,), (0,)), ((), ())), preferred_element_type=F32)


def _nt(a, b):
    return lax.dot_general(a, b, (((1,), (1,)), ((), ())), preferred_element_type=F32)


def _tn(a, b):
    return lax.dot_general(a, b, (((0,), (0,)), ((), ())), preferred_element_type=F32)


def _softmax_pm(p):
    p3 = p.reshape(4, DH, p.shape[-1])
    ep = jnp.exp(p3 - jnp.max(p3, axis=1, keepdims=True))
    em = jnp.exp(jnp.min(p3, axis=1, keepdims=True) - p3)
    sp = ep * (1.0 / jnp.sum(ep, axis=1, keepdims=True))
    sm = em * (1.0 / jnp.sum(em, axis=1, keepdims=True))
    return sp.reshape(p.shape), sm.reshape(p.shape)


def _softmax_pm_bwd(php, phm, dp, dm):
    n = php.shape[-1]
    a, b = php.reshape(4, DH, n), phm.reshape(4, DH, n)
    ta, tb = a * dp.reshape(4, DH, n), b * dm.reshape(4, DH, n)
    r = (ta - tb) - a * jnp.sum(ta, axis=1, keepdims=True) + b * jnp.sum(tb, axis=1, keepdims=True)
    return r.reshape(php.shape)


def _head_mask():
    r = lax.broadcasted_iota(jnp.int32, (128 + EXT, 256), 0)
    c = lax.broadcasted_iota(jnp.int32, (128 + EXT, 256), 1)
    return jnp.where(r < 128, r // DH, r - 128) == (c % 128) // DH


def _finish_state(acc_ref, ext_ref, t_ref, col_ref):
    mask = _head_mask()
    for g in range(G):
        st = jnp.where(mask, acc_ref[g], 0.0).astype(BF)
        ext_ref[g] = st
        st = st.astype(F32)
        t_ref[g] = st[:128].T.astype(BF)
        row = jnp.sum(st[128:], axis=0, keepdims=True)
        col_ref[g] = jnp.broadcast_to(row, (128, 256)).T


def _lanes(col):
    return jnp.concatenate([col] * (T // 128), axis=1)


def _kernel(x_hbm, wqkv_hbm, wphi_ref, wo_hbm, w1_hbm, w2_hbm, go_hbm,
            out_hbm, dx_hbm, dwqkv_hbm, dwphi_ref, dwo_hbm, dw1_hbm, dw2_hbm,
            x_v, go_v, wqkv_v, wo_v, w1_v, w2_v, xn_v, xnT_v, rstd_v, wT_v, bd_v,
            qkvT_v, pkm_v, h_v, ds_v, oT_v, acc_v, ext_v, stT_v, col_v, stage_v,
            sem_x, sem_go, sem_wqkv, sem_wo, sem_w1, sem_w2,
            sem_out, sem_dx, sem_dwqkv, sem_dwo, sem_dw1, sem_dw2):
    cp = pltpu.make_async_copy

    def rows(t):
        return pl.ds(pl.multiple_of(t * T, T), T)

    def x_in(t):
        return cp(x_hbm.at[rows(t), :], x_v.at[rows(t), :], sem_x.at[t])

    def go_in(t):
        return cp(go_hbm.at[rows(t), :], go_v.at[rows(t), :], sem_go.at[t])

    def wqkv_in(i):
        return cp(wqkv_hbm.at[:, pl.ds(i * D, D)], wqkv_v.at[i], sem_wqkv.at[i])

    def w1_in(c):
        return cp(w1_hbm.at[:, pl.ds(c * FC, FC)], w1_v.at[c], sem_w1.at[c])

    def w2_in(c):
        return cp(w2_hbm.at[pl.ds(c * FC, FC), :], w2_v.at[c], sem_w2.at[c])

    wo_in = cp(wo_hbm, wo_v, sem_wo.at[0])

    def out_out(t):
        return cp(x_v.at[rows(t), :], out_hbm.at[rows(t), :], sem_out.at[t])

    def dx_out(t):
        return cp(x_v.at[rows(t), :], dx_hbm.at[rows(t), :], sem_dx.at[t])

    def dwqkv_out(i):
        return cp(wT_v.at[i], dwqkv_hbm.at[:, pl.ds(i * D, D)], sem_dwqkv.at[i])

    def dw1_out(c):
        return cp(stage_v.at[c % 2], dw1_hbm.at[:, pl.ds(pl.multiple_of(c * FC, FC), FC)], sem_dw1.at[c % 2])

    def dw2_out(c):
        return cp(w2_v.at[c], dw2_hbm.at[pl.ds(pl.multiple_of(c * FC, FC), FC), :], sem_dw2.at[c])

    dwo_out = cp(wo_v, dwo_hbm, sem_dwo.at[0])

    for t in range(NT):
        x_in(t).start()
    wqkv_in(1).start()
    wqkv_in(2).start()

    r = lax.broadcasted_iota(jnp.int32, (DH, 128), 0)
    c_ = lax.broadcasted_iota(jnp.int32, (DH, 128), 1)
    rep = _nn(wphi_ref[...], (r == c_ % DH).astype(BF))
    r = lax.broadcasted_iota(jnp.int32, (D, 128), 0)
    c_ = lax.broadcasted_iota(jnp.int32, (D, 128), 1)
    bd_v[...] = jnp.where((r % 128) // DH == c_ // DH, rep, 0.0).astype(BF)

    def ln_body(t, carry):
        x_in(t).wait()
        x = x_v[rows(t), :].astype(F32)
        xc = x - jnp.mean(x, axis=1, keepdims=True)
        rstd = lax.rsqrt(jnp.mean(xc * xc, axis=1, keepdims=True) + 1e-5)
        xn = xc * rstd
        xn_v[rows(t), :] = xn.astype(BF)
        xnT_v[t] = xn.T.astype(BF)
        rstd_v[t] = jnp.broadcast_to(rstd, (T, 128)).T[:8]
        return carry

    lax.fori_loop(0, NT, ln_body, 0)

    wqkv_in(0).start()
    wo_in.start()
    for c in range(NC):
        w1_in(c).start()
        w2_in(c).start()
    for t in range(NT):
        go_in(t).start()

    def prep(i):
        wqkv_in(i).wait()
        r = lax.broadcasted_iota(jnp.int32, (128, 128), 0)
        c_ = lax.broadcasted_iota(jnp.int32, (128, 128), 1)
        for g in range(G):
            gs = slice(g * 128, (g + 1) * 128)
            if i == 2:
                m = (r == c_).astype(BF)
            else:
                m = bd_v[gs, :].astype(F32).T.astype(BF)
            wT_v[i, gs, :] = _nt(m, wqkv_v[i, :, gs]).astype(BF)

    prep(1)
    prep(2)

    acc_v[...] = jnp.zeros(acc_v.shape, F32)

    def p1_body(t, carry):
        xnT = xnT_v[t]
        pk = _nn(wT_v[1], xnT)
        vT = _nn(wT_v[2], xnT).astype(BF)
        qkvT_v[2, t] = vT
        ones = jnp.ones((EXT, T), BF)
        for g in range(G):
            gs = slice(g * 128, (g + 1) * 128)
            sp, sm = _softmax_pm(pk[gs])
            sp, sm = sp.astype(BF), sm.astype(BF)
            qkvT_v[1, t, gs, :] = sp
            pkm_v[t, gs, :] = sm
            acc_v[g] += _nt(jnp.concatenate([vT[gs], ones], axis=0), jnp.concatenate([sp, sm], axis=0))
        return carry

    lax.fori_loop(0, NT, p1_body, 0)
    _finish_state(acc_v, ext_v, stT_v, col_v)
    acc_v[...] = jnp.zeros(acc_v.shape, F32)

    prep(0)
    wo_in.wait()
    for c in range(NC):
        w1_in(c).wait()
        w2_in(c).wait()

    def p2_body(t, carry):
        go_in(t).wait()
        xnT = xnT_v[t]
        pq = _nn(wT_v[0], xnT)
        phis, os_, rdens = [], [], []
        for g in range(G):
            gs = slice(g * 128, (g + 1) * 128)
            sp, sm = _softmax_pm(pq[gs])
            phi = jnp.concatenate([sp.astype(BF), sm.astype(BF)], axis=0)
            nd = _nn(ext_v[g], phi)
            rd = 1.0 / (nd[128:136] + 1e-6)
            rden = jnp.concatenate(
                [jnp.broadcast_to(rd[j:j + 1], (DH, T)) for j in range(4)], axis=0)
            o = nd[:128] * rden
            oT_v[t, gs, :] = o.astype(BF)
            phis.append(phi)
            os_.append(o)
            rdens.append(rden)
        o_tok = jnp.concatenate([o.T.astype(BF) for o in os_], axis=1)
        s = _nn(o_tok, wo_v[...])

        xn = xn_v[rows(t), :]
        m = None
        for c in range(NC):
            h = _nn(xn, w1_v[c]).astype(BF)
            h_v[c, rows(t), :] = h
            mc = _nn(jnp.maximum(h, 0), w2_v[c])
            m = mc if m is None else m + mc
        sig = 1.0 / (1.0 + jnp.exp(-m))
        gate = m * sig
        go = go_v[rows(t), :].astype(F32)
        x_v[rows(t), :] = (x_v[rows(t), :].astype(F32) + s * gate).astype(BF)
        out_out(t).start()
        ds = (go * gate).astype(BF)
        ds_v[rows(t), :] = ds
        xn_v[rows(t), :] = (go * s * (sig + gate * (1.0 - sig))).astype(BF)

        doT = _nt(wo_v[...], ds)
        sub = lax.broadcasted_iota(jnp.int32, (EXT, T), 0)
        for g in range(G):
            gs = slice(g * 128, (g + 1) * 128)
            dnum = doT[gs] * rdens[g]
            tt = dnum * os_[g]
            dd = [-jnp.sum(tt[j * DH:(j + 1) * DH], axis=0, keepdims=True) for j in range(4)]
            dden_ext = jnp.zeros((EXT, T), F32)
            for j in range(4):
                dden_ext = jnp.where(sub == j, jnp.broadcast_to(dd[j], (EXT, T)), dden_ext)
            dden = jnp.concatenate([jnp.broadcast_to(dd[j], (DH, T)) for j in range(4)], axis=0)
            dnum = dnum.astype(BF)
            phi = phis[g]
            acc_v[g] += _nt(jnp.concatenate([dnum, dden_ext.astype(BF)], axis=0), phi)
            dphi = _nn(stT_v[g], dnum)
            col = col_v[g]
            dpq = _softmax_pm_bwd(phi[:128].astype(F32), phi[128:].astype(F32),
                                  dphi[:128] + _lanes(col[:128]) * dden,
                                  dphi[128:] + _lanes(col[128:]) * dden)
            qkvT_v[0, t, gs, :] = dpq.astype(BF)
        return carry

    lax.fori_loop(0, NT, p2_body, 0)
    _finish_state(acc_v, ext_v, stT_v, col_v)

    def p3_body(c, carry):
        dm = xn_v[...]
        da = _nt(dm, w2_v[c])
        h = h_v[c]
        hf = h.astype(F32)
        dh = (da * jnp.where(hf > 0, 1.0, jnp.where(hf == 0, 0.5, 0.0))).astype(BF)
        w2_v[c] = _tn(jnp.maximum(h, 0), dm).astype(BF)
        dw2_out(c).start()
        h_v[c] = dh
        dw1 = None
        for t in range(NT):
            p = _nn(xnT_v[t], dh[t * T:(t + 1) * T])
            dw1 = p if dw1 is None else dw1 + p

        @pl.when(c >= 2)
        def _():
            dw1_out(c - 2).wait()

        stage_v[c % 2] = dw1.astype(BF)
        dw1_out(c).start()
        return carry

    lax.fori_loop(0, NC, p3_body, 0)

    dwo = None
    for t in range(NT):
        p = _nn(oT_v[t], ds_v[t * T:(t + 1) * T, :])
        dwo = p if dwo is None else dwo + p
    wo_v[...] = dwo.astype(BF)
    dwo_out.start()

    def p4_body(t, carry):
        for g in range(G):
            gs = slice(g * 128, (g + 1) * 128)
            php, phm = qkvT_v[1, t, gs, :], pkm_v[t, gs, :]
            v = qkvT_v[2, t, gs, :]
            dv = _nn(ext_v[g, :128, :], jnp.concatenate([php, phm], axis=0))
            dphi = _nn(stT_v[g], v)
            col = col_v[g]
            dpk = _softmax_pm_bwd(php.astype(F32), phm.astype(F32),
                                  dphi[:128] + _lanes(col[:128]), dphi[128:] + _lanes(col[128:]))
            qkvT_v[1, t, gs, :] = dpk.astype(BF)
            qkvT_v[2, t, gs, :] = dv.astype(BF)
        return carry

    lax.fori_loop(0, NT, p4_body, 0)

    def proj_grad(i):
        acc = None
        for t in range(NT):
            p = _nt(xnT_v[t], qkvT_v[i, t])
            acc = p if acc is None else acc + p
        return acc.astype(BF)

    acc_v[...] = jnp.zeros(acc_v.shape, F32)

    def p5_body(i, carry):
        gi = proj_grad(i)
        for g in range(G):
            gs = slice(g * 128, (g + 1) * 128)
            bd = bd_v[gs, :]
            w = wqkv_v[i, :, gs]
            wT_v[i, :, gs] = _nt(gi[:, gs], bd).astype(BF)
            acc_v[g, :128, :128] += _tn(w, gi[:, gs])
            wqkv_v[i, :, gs] = _nn(w, bd).astype(BF)
        return carry

    lax.fori_loop(0, 2, p5_body, 0)
    dwqkv_out(0).start()
    dwqkv_out(1).start()
    wT_v[2] = proj_grad(2)
    dwqkv_out(2).start()
    for g in range(G):
        for j in range(4):
            hs = slice(j * DH, (j + 1) * DH)
            dwphi_ref[g * 128 + j * DH:g * 128 + (j + 1) * DH, :] = acc_v[g, hs, :128][:, hs].astype(BF)

    def p6_body(t, carry):
        d = None
        for i in range(3):
            p = _nn(wqkv_v[i], qkvT_v[i, t])
            d = p if d is None else d + p
        for c in range(NC):
            d = d + _nt(w1_v[c], h_v[c, rows(t), :])
        xnT = xnT_v[t].astype(F32)
        m1 = jnp.mean(d, axis=0, keepdims=True)
        m2 = jnp.mean(d * xnT, axis=0, keepdims=True)
        dxT = (d - m1 - xnT * m2) * rstd_v[t][0:1]
        out_out(t).wait()
        x_v[rows(t), :] = (go_v[rows(t), :].astype(F32) + dxT.T).astype(BF)
        dx_out(t).start()
        return carry

    lax.fori_loop(0, NT, p6_body, 0)

    for c in range(NC):
        dw2_out(c).wait()
    dw1_out(NC - 2).wait()
    dw1_out(NC - 1).wait()
    dwo_out.wait()
    for i in range(3):
        dwqkv_out(i).wait()
    for t in range(NT):
        dx_out(t).wait()


@jax.jit
def pallas_recurrent_scan__linear_kernel_hedgehog__dense_activation_relu__prompt_kernel(
    A_x: jax.Array,
    A_wqkv: jax.Array,
    A_w_phi: jax.Array,
    A_wo: jax.Array,
    B_x: jax.Array,
    B_w1: jax.Array,
    B_w2: jax.Array,
    grad_out: jax.Array,
):
    del B_x
    hbm = pl.BlockSpec(memory_space=pl.ANY)
    vmem = pl.BlockSpec(memory_space=pltpu.VMEM)
    sds = jax.ShapeDtypeStruct
    V = pltpu.VMEM
    dma = pltpu.SemaphoreType.DMA
    out, dx, dwqkv, dwphi, dwo, dw1, dw2 = pl.pallas_call(
        _kernel,
        in_specs=[hbm, hbm, vmem, hbm, hbm, hbm, hbm],
        out_specs=[hbm, hbm, hbm, vmem, hbm, hbm, hbm],
        out_shape=[sds((S, D), BF), sds((S, D), BF), sds((D, 3 * D), BF), sds((D, DH), BF),
                   sds((D, D), BF), sds((D, F), BF), sds((F, D), BF)],
        scratch_shapes=[
            V((S, D), BF), V((S, D), BF), V((3, D, D), BF), V((D, D), BF),
            V((NC, D, FC), BF), V((NC, FC, D), BF),
            V((S, D), BF), V((NT, D, T), BF), V((NT, 8, T), F32), V((3, D, D), BF), V((D, 128), BF),
            V((3, NT, D, T), BF), V((NT, D, T), BF), V((NC, S, FC), BF), V((S, D), BF), V((NT, D, T), BF),
            V((G, 128 + EXT, 256), F32), V((G, 128 + EXT, 256), BF), V((G, 256, 128), BF),
            V((G, 256, 128), F32), V((2, D, FC), BF),
            dma((NT,)), dma((NT,)), dma((3,)), dma((1,)), dma((NC,)), dma((NC,)),
            dma((NT,)), dma((NT,)), dma((3,)), dma((1,)), dma((2,)), dma((NC,)),
        ],
        compiler_params=pltpu.CompilerParams(vmem_limit_bytes=126 * 1024 * 1024),
    )(A_x.reshape(S, D), A_wqkv, A_w_phi.reshape(D, DH), A_wo, B_w1, B_w2, grad_out.reshape(S, D))
    return (out.reshape(1, S, D), dx.reshape(1, S, D), dwqkv, dwphi.reshape(H, DH, DH), dwo, dw1, dw2)
```

```python
import jax
import jax.numpy as jnp
from jax import lax
import jax.experimental.pallas as pl
import jax.experimental.pallas.tpu as pltpu

S, D, H, F = 2048, 1024, 32, 3584
DH = D // H
T = 512
NT = S // T
FC = 512
NC = F // FC
G = D // 128
HS, HD, HF, TH, GH = S // 2, D // 2, FC // 2, T // 2, 3 * G // 2
PR = 2 * DH
EXT = 16
BF, F32 = jnp.bfloat16, jnp.float32


def _nn(a, b):
    return lax.dot_general(a, b, (((1,), (0,)), ((), ())), preferred_element_type=F32)


def _nt(a, b):
    return lax.dot_general(a, b, (((1,), (1,)), ((), ())), preferred_element_type=F32)


def _tn(a, b):
    return lax.dot_general(a, b, (((0,), (0,)), ((), ())), preferred_element_type=F32)


def _sums(q11, q12, q21, q22):
    a, b, c, d = (q.astype(F32) for q in (q11, q12, q21, q22))
    return [v.astype(BF) for v in (a + d, c + d, a + b, c - a, b - d)]


def _lazy(q):
    f = lambda k: q(k).astype(F32)
    return (lambda: q(0), lambda: q(3),
            [lambda: (f(0) + f(3)).astype(BF), lambda: (f(2) + f(3)).astype(BF), lambda: (f(0) + f(1)).astype(BF),
             lambda: (f(2) - f(0)).astype(BF), lambda: (f(1) - f(3)).astype(BF)])


def _as_lhs(q11, q22, s):
    return [s[0], s[1], q11, q22, s[2], s[3], s[4]]


def _as_rhs(q11, q22, s):
    return [s[0], q11, s[4], s[3], q22, s[2], s[1]]


_USES = ({0: 1, 3: 1}, {2: 1, 3: -1}, {1: 1, 3: 1}, {0: 1, 2: 1}, {0: -1, 1: 1}, {3: 1}, {0: 1})


def _strassen(dot, a, b, done=lambda k, v: v, fill=(), order=(1, 3, 4, 2, 0, 6, 5)):
    get = lambda v: v() if callable(v) else v
    c, left = {}, [4, 2, 2, 4]
    for n, i in enumerate(order):
        m = dot(get(a[i]), get(b[i]))
        if n < len(fill):
            fill[n]()
        for k, sign in _USES[i].items():
            if k not in c:
                c[k] = (sign, m)
            else:
                c[k] = (1, m - c[k][1] if c[k][0] < 0 else c[k][1] + m if sign > 0 else c[k][1] - m)
            left[k] -= 1
            if not left[k]:
                c[k] = done(k, c[k][1])
    return [c[k] for k in range(4)]


def _softmax_pm(p):
    p3 = p.reshape(-1, DH, p.shape[-1])
    ep = jnp.exp(p3 - jnp.max(p3, axis=1, keepdims=True))
    em = jnp.exp(jnp.min(p3, axis=1, keepdims=True) - p3)
    sp = ep * (1.0 / jnp.sum(ep, axis=1, keepdims=True))
    sm = em * (1.0 / jnp.sum(em, axis=1, keepdims=True))
    return sp.reshape(p.shape), sm.reshape(p.shape)


def _softmax_pm_bwd(php, phm, dp, dm):
    n = php.shape[-1]
    a, b = php.reshape(-1, DH, n), phm.reshape(-1, DH, n)
    ta, tb = a * dp.reshape(-1, DH, n), b * dm.reshape(-1, DH, n)
    r = (ta - tb) - a * jnp.sum(ta, axis=1, keepdims=True) + b * jnp.sum(tb, axis=1, keepdims=True)
    return r.reshape(php.shape)


def _finish_state(acc_ref, ext_ref, t_ref, col_ref):
    r = lax.broadcasted_iota(jnp.int32, (PR + EXT, 128), 0)
    c = lax.broadcasted_iota(jnp.int32, (PR + EXT, 128), 1)
    mask = jnp.where(r < PR, r // DH, r - PR) == (c % PR) // DH
    zero = jnp.zeros((PR, 128), F32)
    for p in range(2 * G):
        st = jnp.where(mask, acc_ref[p], 0.0).astype(BF)
        acc_ref[p] = jnp.zeros((PR + EXT, 128), F32)
        ext_ref[p] = st
        st = st.astype(F32)
        t_ref[p] = jnp.concatenate([st[:PR], zero][::1 - 2 * (p % 2)], axis=0).T.astype(BF)
        col_ref[p] = jnp.broadcast_to(jnp.sum(st[PR:], axis=0, keepdims=True), (128, 128)).T


def _pair(plus, minus, i):
    return jnp.concatenate([plus[_half(i, PR)], minus[_half(i, PR)]], axis=0)


def _lanes(col):
    return jnp.concatenate([col] * (T // 128), axis=1)


def _normalize(x):
    x = x.astype(F32)
    xc = x - jnp.mean(x, axis=1, keepdims=True)
    rstd = lax.rsqrt(jnp.mean(xc * xc, axis=1, keepdims=True) + 1e-5)
    return xc * rstd, rstd


def _half(i, n):
    return slice(i * n, (i + 1) * n)


def _kernel(x_hbm, wqkv_hbm, wphi_ref, wo_hbm, w1_hbm, w2_hbm, go_hbm,
            out_hbm, dx_hbm, dwqkv_hbm, dwphi_ref, dwo_hbm, dw1_hbm, dw2_hbm,
            x_v, go_v, wo_v, w1_v, w2_v, xn_v, xnT_v, wT_v, bd_v,
            qkvT_v, pkm_v, h_v, oT_v, rd_v, m_v, acc_v, ext_v, stT_v, col_v, ts_v, fs_v, wos_v,
            sem_x, sem_go, sem_wqkv, sem_wo, sem_w1, sem_w2,
            sem_out, sem_dx, sem_dwqkv, sem_dwo, sem_dw1, sem_dw2):
    cp = pltpu.make_async_copy

    def rows(t, j):
        return pl.ds(pl.multiple_of(j * HS + t * TH, TH), TH)

    def qrows(t):
        return pl.ds(pl.multiple_of(t * TH, TH), TH)

    def tile_cp(src, dst, sem, t):
        return [cp(src.at[rows(t, j), :], dst.at[rows(t, j), :], sem.at[2 * t + j]) for j in range(2)]

    def start(cs):
        for c in cs:
            c.start()

    def wait(cs):
        for c in cs:
            c.wait()

    def tile(ref, t):
        return jnp.concatenate([ref[rows(t, 0), :], ref[rows(t, 1), :]], axis=0)

    def set_tile(ref, t, v):
        ref[rows(t, 0), :] = v[:TH]
        ref[rows(t, 1), :] = v[TH:]

    def fquad(ref, i, j):
        return jnp.concatenate([ref[t, _half(i, HD), _half(j, TH)] for t in range(NT)], axis=1)

    def xnT_lhs():
        return _as_lhs(lambda: fquad(xnT_v, 0, 0), lambda: fquad(xnT_v, 1, 1),
                       [lambda k=k: jnp.concatenate([fs_v[k, t] for t in range(NT)], axis=1) for k in range(5)])

    x_in = lambda t: tile_cp(x_hbm, x_v, sem_x, t)
    go_in = lambda t: tile_cp(go_hbm, go_v, sem_go, t)
    out_out = lambda t: tile_cp(x_v, out_hbm, sem_out, t)
    dx_out = lambda t: tile_cp(xn_v, dx_hbm, sem_dx, t)

    def wqkv_in(k):
        return cp(wqkv_hbm.at[:, fcols(k)], qkvT_v.at[k // 2, k % 2], sem_wqkv.at[k])

    def wqkv_again(k):
        return cp(wqkv_hbm.at[:, fcols(k)], w1_v.at[k], sem_wqkv.at[k])

    def fcols(c):
        return pl.ds(pl.multiple_of(c * FC, FC), FC)

    def w_in(c):
        return [cp(w1_hbm.at[:, fcols(c)], w1_v.at[c], sem_w1.at[c]),
                cp(w2_hbm.at[fcols(c), :], w2_v.at[c], sem_w2.at[c])]

    def dw1_out(c):
        return cp(h_v.at[c, :D, :], dw1_hbm.at[:, fcols(c)], sem_dw1.at[c])

    def dw2_out(c):
        return cp(w2_v.at[c], dw2_hbm.at[fcols(c), :], sem_dw2.at[c])

    def dwqkv_out(k):
        return cp(wT_v.at[k], dwqkv_hbm.at[:, fcols(k)], sem_dwqkv.at[k])

    def dwv_out(j):
        return cp(pkm_v.at[j], dwqkv_hbm.at[:, fcols(4 + j)], sem_dwqkv.at[4 + j])

    wo_in = cp(wo_hbm, wo_v, sem_wo.at[0])
    dwo_out = cp(wo_v, dwo_hbm, sem_dwo.at[0])

    def token_sums(t, v):
        for k, u in enumerate(_sums(v[:TH, :HD], v[:TH, HD:], v[TH:, :HD], v[TH:, HD:])):
            ts_v[k, qrows(t), :] = u

    for t in range(NT):
        start(x_in(t))
    start(w_in(0))

    r = lax.broadcasted_iota(jnp.int32, (DH, 128), 0)
    c_ = lax.broadcasted_iota(jnp.int32, (DH, 128), 1)
    rep = _nn(wphi_ref[...], (r == c_ % DH).astype(BF))
    r = lax.broadcasted_iota(jnp.int32, (D, 128), 0)
    c_ = lax.broadcasted_iota(jnp.int32, (D, 128), 1)
    bd_v[...] = jnp.where((r % 128) // DH == c_ // DH, rep, 0.0).astype(BF)

    m_v[...] = jnp.zeros(m_v.shape, F32)
    acc_v[...] = jnp.zeros(acc_v.shape, F32)

    def ln_body(t, carry):
        wait(x_in(t))
        xn, _ = _normalize(tile(x_v, t))
        set_tile(xn_v, t, xn.astype(BF))
        token_sums(t, xn)
        for g in range(4):
            q = [xn_v[rows(t, k % 2), _half(4 * (k // 2) + g, 128)].T for k in range(4)]
            for k in range(4):
                xnT_v[t, _half(4 * (k // 2) + g, 128), _half(k % 2, TH)] = q[k]
            for k, u in enumerate(_sums(*q)):
                fs_v[k, t, _half(g, 128), :] = u
        return carry

    with jax.named_scope('ln'):
        lax.fori_loop(0, NT, ln_body, 0)

    def quads(ref, c, nr, nc):
        return [ref[c, _half(k // 2, nr), _half(k % 2, nc)] for k in range(4)]

    def tok_ops(side):
        return side(lambda: xn_v[:HS, :HD], lambda: xn_v[HS:, HD:], [lambda k=k: ts_v[k] for k in range(5)])

    def add_m(k, v):
        m_v[k] += v

    def put(ref, nr, nc):
        def store(k, v):
            ref[_half(k // 2, nr), _half(k % 2, nc)] = v.astype(BF)
        return store

    tall = lambda ref: [ref.at[k // 2, :, _half(k % 2, HF)] for k in range(7)]

    def ff_body(c, carry):
        wait(w_in(c))

        @pl.when(c < NC - 1)
        def _():
            start(w_in(c + 1))
            wqkv_in(c).start()

        w = quads(w1_v, c, HD, HF)

        def act(k, h):
            h = h.astype(BF)
            h_v[c, _half(k // 2, HS), _half(k % 2, HF)] = h
            tall(oT_v)[k][...] = jnp.maximum(h, 0)

        _strassen(_nn, tok_ops(_as_lhs), _as_rhs(w[0], w[3], _sums(*w)), act)
        w = quads(w2_v, c, HF, HD)
        _strassen(_nn, _as_lhs(*_lazy(lambda k: tall(oT_v)[k][...])), _as_rhs(w[0], w[3], _sums(*w)), add_m,
                  order=(2, 4, 5, 3, 1, 0, 6))
        return carry

    wo_in.start()
    with jax.named_scope('ff'):
        lax.fori_loop(0, NC, ff_body, 0)

    slots = ([ts_v.at[k // 2, _half(k % 2, HD), :] for k in range(10)]
             + [oT_v.at[k // 2, _half(k % 2, HD), :] for k in range(8)]
             + [xn_v.at[_half(k, HD), :HD] for k in range(3)])

    def w_rows(g):
        w = qkvT_v[g // G, g % G // 4, :, _half(g % 4, 128)]
        return w.T if g // G == 2 else _nt(bd_v[_half(g % G, 128), :].T, w)

    with jax.named_scope('prep'):
        for k in range(6):
            wqkv_in(k).wait()
        wo_in.wait()
        for t in range(NT):
            start(go_in(t))
        for k, u in enumerate(_sums(wo_v[:HD, :HD], wo_v[:HD, HD:], wo_v[HD:, :HD], wo_v[HD:, HD:])):
            wos_v[k] = u
        for g in (0, 4, 8, 1, 5, 9, 2, 6, 10, 3, 7, 11):
            top, bot = w_rows(g // 4 * G + g % 4), w_rows(g // 4 * G + g % 4 + 4)
            ops = _as_lhs(top[:, :HD].astype(BF), bot[:, HD:].astype(BF),
                          _sums(top[:, :HD], top[:, HD:], bot[:, :HD], bot[:, HD:]))
            for k in range(7):
                slots[3 * k + g // 4][_half(g % 4, 128), :] = ops[k]


    def p1_body(t, carry):
        q = _strassen(_nn, [lambda k=k: jnp.concatenate([v[...] for v in slots[3 * k:3 * k + 3]], axis=0) for k in range(7)],
                      _as_rhs(xnT_v[t, :HD, :TH], xnT_v[t, HD:, TH:], [fs_v[k, t] for k in range(5)]))

        def proj(g):
            rs, hi = _half(g // G * 4 + g % 4, 128), g % G // 4
            return jnp.concatenate([q[2 * hi][rs], q[2 * hi + 1][rs]], axis=1)

        ones = jnp.ones((EXT, T), BF)
        for g in (4, 5, 6, 7, 0, 1, 2, 3):
            gs = _half(g, 128)
            sp, sm = _softmax_pm(proj(g))
            qkvT_v[0, t, gs, :] = sp.astype(BF)
            wT_v[t, gs, :] = sm.astype(BF)
            sp, sm = _softmax_pm(proj(G + g))
            sp, sm = sp.astype(BF), sm.astype(BF)
            v = proj(2 * G + g).astype(BF)
            qkvT_v[1, t, gs, :] = sp
            pkm_v[t, gs, :] = sm
            qkvT_v[2, t, gs, :] = v
            for i in range(2):
                acc_v[2 * g + i] += _nt(jnp.concatenate([v[_half(i, PR)], ones], axis=0), _pair(sp, sm, i))
        return carry

    with jax.named_scope('p1'):
        lax.fori_loop(0, NT, p1_body, 0)
    _finish_state(acc_v, ext_v, stT_v, col_v)

    def head_rows(v):
        return jnp.concatenate([jnp.broadcast_to(v[j:j + 1], (DH, T)) for j in range(2)], axis=0)

    def phi_q(t, p):
        return jnp.concatenate([qkvT_v[0, t, _half(p, PR), :], wT_v[t, _half(p, PR), :]], axis=0)

    def state_T(g):
        return jnp.concatenate([stT_v[2 * g], stT_v[2 * g + 1]], axis=0)

    def p2_body(t, carry):
        wait(go_in(t))
        o_tok, gate, dgate, ds = [], {}, {}, {}
        for g in range(G):
            gs = _half(g, 128)
            o = []
            for p in (2 * g, 2 * g + 1):
                nd = _nn(ext_v[p], phi_q(t, p))
                rd = 1.0 / (nd[PR:PR + 8] + 1e-6)
                rd_v[p] = rd
                o.append(nd[:PR] * head_rows(rd))
            o = jnp.concatenate(o, axis=0)
            oT_v[t, gs, :] = o.astype(BF)
            o_tok.append(o.astype(BF).T)
            k, cs = g // 2, _half(g % 2, HD // 2)
            at = (rows(t, k // 2), _half(2 * (k % 2) + g % 2, HD // 2))
            m = m_v[k, qrows(t), cs]
            sig = 1.0 / (1.0 + jnp.exp(-m))
            go = go_v[at].astype(F32)
            gate[g] = m * sig
            dgate[g] = go * (sig + gate[g] * (1.0 - sig))
            ds[g] = (go * gate[g]).astype(BF)
            go_v[at] = ds[g]
        gate, dgate, ds = ([jnp.concatenate([v[2 * k], v[2 * k + 1]], axis=1) for k in range(4)]
                           for v in (gate, dgate, ds))
        wo = (lambda: wo_v[:HD, :HD], lambda: wo_v[HD:, HD:], [lambda k=k: wos_v[k] for k in range(5)])
        do = _strassen(_nt, _as_lhs(*wo), _as_rhs(ds[0], ds[3], _sums(ds[0], ds[2], ds[1], ds[3])))
        sub = lax.broadcasted_iota(jnp.int32, (EXT, T), 0)

        def group_bwd(g):
            gs = _half(g, 128)
            dnum = jnp.concatenate([v[_half(g % 4, 128)] for v in do[_half(g // 4, 2)]], axis=1)
            dnum = dnum * jnp.concatenate([head_rows(rd_v[2 * g]), head_rows(rd_v[2 * g + 1])], axis=0)
            tt = dnum * oT_v[t, gs, :].astype(F32)
            dnum = dnum.astype(BF)
            dphis = _nn(state_T(g), dnum)
            for i in range(2):
                p = 2 * g + i
                dd = [-jnp.sum(tt[_half(2 * i + j, DH)], axis=0, keepdims=True) for j in range(2)]
                dden_ext = jnp.where(sub == 0, jnp.broadcast_to(dd[0], (EXT, T)), jnp.broadcast_to(dd[1], (EXT, T)))
                dden = jnp.concatenate([jnp.broadcast_to(dd[j % 2], (DH, T)) for j in range(4)], axis=0)
                phi = phi_q(t, p)
                acc_v[p] += _nt(jnp.concatenate([dnum[_half(i, PR)], dden_ext.astype(BF)], axis=0), phi)
                dphi = dphis[_half(i, 128)] + _lanes(col_v[p]) * dden
                phi = phi.astype(F32)
                qkvT_v[0, t, _half(p, PR), :] = _softmax_pm_bwd(phi[:PR], phi[PR:], dphi[:PR], dphi[PR:]).astype(BF)

        def gated(k, s):
            at = (rows(t, k // 2), _half(k % 2, HD))
            x_v[at] = (x_v[at].astype(F32) + s * gate[k]).astype(BF)
            dm = (s * dgate[k]).astype(BF)
            xn_v[at] = dm
            m_v[k, qrows(t), :] = jnp.zeros((TH, HD), F32)
            return dm

        o = [jnp.concatenate([v[_half(k // 2, TH)] for v in o_tok[_half(k % 2, 4)]], axis=1) for k in range(4)]
        o = _as_lhs(o[0], o[3], _sums(*o))
        group_bwd(0)
        group_bwd(1)
        dm = _strassen(_nn, o, _as_rhs(*wo), gated, [lambda g=g: group_bwd(g) for g in range(2, G)])
        for k, u in enumerate(_sums(*dm)):
            ts_v[k, qrows(t), :] = u
        start(out_out(t))
        return carry

    with jax.named_scope('p2'):
        lax.fori_loop(0, NT, p2_body, 0)

    _finish_state(acc_v, ext_v, stT_v, col_v)

    def p3a_body(c, carry):
        def act_bwd(k, da, p):
            at = (c, _half(2 * (k // 2) + p, HD), _half(k % 2, HF))
            h = h_v[at].astype(F32)
            h_v[at] = (da[_half(p, HD)] * jnp.where(h > 0, 1.0, jnp.where(h == 0, 0.5, 0.0))).astype(BF)

        def early(k, da):
            if k == 1:
                act_bwd(k, da, 0)
                act_bwd(k, da, 1)
            return da

        def flip(p):
            q = [jnp.maximum(h_v[c, _half(4 * (k % 2) + p, HF), _half(k // 2, HF)], 0).T for k in range(4)]
            for k, v in enumerate([q[0], q[3]] + _sums(*q)):
                wT_v[k // 2, _half(2 * (k % 2) + p // 2, HF), _half(p % 2, HF)] = v

        aT = [lambda k=k: jnp.concatenate([wT_v[k // 2, _half(2 * (k % 2) + p, HF), :] for p in range(2)], axis=1)
              for k in range(7)]
        w = quads(w2_v, c, HF, HD)
        da = _strassen(_nt, tok_ops(_as_lhs), _as_rhs(w[0], w[3], _sums(w[0], w[2], w[1], w[3])), early,
                       [lambda: (flip(0), flip(1)), lambda: flip(2), lambda: flip(3)])
        _strassen(_nn, _as_lhs(aT[0], aT[1], aT[2:]), tok_ops(_as_rhs),
                  put(w2_v.at[c], HF, HD),
                  [lambda k=k, p=p: act_bwd(k, da[k], p) for k in (2, 0, 3) for p in range(2)])
        dw2_out(c).start()
        return carry

    with jax.named_scope('p3a'):
        lax.fori_loop(0, NC, p3a_body, 0)

    for t in range(NT):
        wait(out_out(t))
        start(x_in(t))

    def p3_body(c, carry):
        q11, q22, sums = _lazy(lambda k: h_v[c, _half(k // 2, HS), _half(k % 2, HF)])
        sums.append(q11)
        views = tall(wT_v)

        def keep(k):
            views[k][...] = sums[k]()

        dh = (lambda: views[5][...], q22, [lambda v=v: v[...] for v in views])
        keep(1)
        w = quads(w1_v, c, HD, HF)
        _strassen(_nt, _as_lhs(*dh), _as_rhs(w[0], w[3], _sums(w[0], w[2], w[1], w[3])), add_m,
                  [lambda k=k: keep(k) for k in (2, 5, 0, 4, 3)])
        _strassen(_nn, xnT_lhs(), _as_rhs(*dh), put(h_v.at[c], HD, HF))
        dw1_out(c).start()
        return carry

    with jax.named_scope('p3'):
        lax.fori_loop(0, NC, p3_body, 0)

    for k in range(6):
        wqkv_again(k).start()
    with jax.named_scope('dwo'):
        o = _lazy(lambda k: fquad(oT_v, k // 2, k % 2))
        d = _lazy(lambda k: go_v[_half(k // 2, HS), _half(k % 2, HD)])
        _strassen(_nn, _as_lhs(*o), _as_rhs(*d), put(wo_v, HD, HD))
    dwo_out.start()
    for t in range(NT):
        start(go_in(t))

    def p4_body(t, carry):
        for g in range(G):
            gs = _half(g, 128)
            dphis = _nn(state_T(g), qkvT_v[2, t, gs, :])
            for i in range(2):
                p = 2 * g + i
                ps = _half(p, PR)
                php, phm = qkvT_v[1, t, ps, :], pkm_v[t, ps, :]
                dv = _nn(ext_v[p, :PR, :], jnp.concatenate([php, phm], axis=0))
                dphi = dphis[_half(i, 128)] + _lanes(col_v[p])
                dpk = _softmax_pm_bwd(php.astype(F32), phm.astype(F32), dphi[:PR], dphi[PR:])
                qkvT_v[1, t, ps, :] = dpk.astype(BF)
                qkvT_v[2, t, ps, :] = dv.astype(BF)
        return carry

    with jax.named_scope('p4'):
        lax.fori_loop(0, NT, p4_body, 0)

    def proj_grad(i):
        b = _lazy(lambda k: fquad(qkvT_v.at[i], k % 2, k // 2))
        q = _strassen(_nt, xnT_lhs(), _as_rhs(*b), lambda k, v: v.astype(BF))
        return [jnp.concatenate([q[j], q[2 + j]], axis=0) for j in range(2)]

    def put_w(i, w):
        ops = _as_lhs(w[0][:HD].astype(BF), w[1][HD:].astype(BF), _sums(w[0][:HD], w[1][:HD], w[0][HD:], w[1][HD:]))
        for k in range(7):
            h_v[k, pl.ds(pl.multiple_of(i * HD, HD), HD), :] = ops[k]

    col_v[:G] = jnp.zeros((G, 128, 128), F32)

    def p5_body(i, carry):
        gi = proj_grad(i)
        for j in range(2):
            pkm_v[j] = gi[j]

        @pl.when(i < 2)
        def _():
            folded = []
            for g in range(G):
                gs, ls = _half(g, 128), _half(g % 4, 128)
                bd, w, gg = bd_v[gs, :], w1_v[2 * i + g // 4, :, ls], pkm_v[g // 4, :, ls]
                wT_v[2 * i + g // 4, :, ls] = _nt(gg, bd).astype(BF)
                col_v[g] += _tn(w, gg)
                folded.append(_nn(w, bd))
            put_w(i, [jnp.concatenate(folded[:4], axis=1), jnp.concatenate(folded[4:], axis=1)])
            for j in range(2):
                dwqkv_out(2 * i + j).start()

        return carry

    for k in range(6):
        wqkv_again(k).wait()
    for c in range(NC):
        dw1_out(c).wait()
    with jax.named_scope('p5'):
        lax.fori_loop(0, 3, p5_body, 0)
    with jax.named_scope('p5v'):
        for j in range(2):
            dwv_out(j).start()
        put_w(2, [w1_v[4], w1_v[5]])
        for g in range(G):
            for j in range(4):
                hs = _half(j, DH)
                dwphi_ref[_half(4 * g + j, DH), :] = col_v[g, hs, :][:, hs].astype(BF)

    def ln_bwd(t, j, p):
        r0 = pl.multiple_of(t * TH + p * 128, 128)
        at = pl.ds(pl.multiple_of(j * HS + r0, 128), 128)
        d = jnp.concatenate([m_v[2 * j + i, pl.ds(r0, 128), :] for i in range(2)], axis=1)
        xn, rstd = _normalize(x_v[at, :])
        m1 = jnp.mean(d, axis=1, keepdims=True)
        m2 = jnp.mean(d * xn, axis=1, keepdims=True)
        xn_v[at, :] = (go_v[at, :].astype(F32) + (d - m1 - xn * m2) * rstd).astype(BF)

    def p6_body(t, carry):
        b = _lazy(lambda k: jnp.concatenate(
            [qkvT_v[i, t, _half(k // 2, HD), _half(k % 2, TH)] for i in range(3)], axis=0))
        a = [lambda k=k: jnp.concatenate([h_v[k, _half(i, HD), :] for i in range(3)], axis=1) for k in range(7)]

        def finish(k, v):
            m_v[2 * (k % 2) + k // 2, qrows(t), :] += v.astype(BF).T.astype(F32)

        _strassen(_nn, a, _as_rhs(*b), finish,
                  [lambda: None] + [lambda j=j, p=p: ln_bwd(jnp.maximum(t - 1, 0), j, p) for j in range(2) for p in range(2)])

        @pl.when(t > 0)
        def _():
            start(dx_out(t - 1))

        return carry

    for t in range(NT):
        wait(x_in(t))
        wait(go_in(t))
    with jax.named_scope('p6'):
        lax.fori_loop(0, NT, p6_body, 0)
    for j in range(2):
        for p in range(2):
            ln_bwd(NT - 1, j, p)
        dx_out(NT - 1)[j].start()

    for c in range(NC):
        dw2_out(c).wait()
    dwo_out.wait()
    for k in range(4):
        dwqkv_out(k).wait()
    for j in range(2):
        dwv_out(j).wait()
    for t in range(NT):
        wait(dx_out(t))


@jax.jit
def pallas_recurrent_scan__linear_kernel_hedgehog__dense_activation_relu__prompt_kernel(
    A_x: jax.Array,
    A_wqkv: jax.Array,
    A_w_phi: jax.Array,
    A_wo: jax.Array,
    B_x: jax.Array,
    B_w1: jax.Array,
    B_w2: jax.Array,
    grad_out: jax.Array,
):
    del B_x
    hbm = pl.BlockSpec(memory_space=pl.ANY)
    vmem = pl.BlockSpec(memory_space=pltpu.VMEM)
    sds = jax.ShapeDtypeStruct
    V = pltpu.VMEM
    dma = pltpu.SemaphoreType.DMA
    out, dx, dwqkv, dwphi, dwo, dw1, dw2 = pl.pallas_call(
        _kernel,
        in_specs=[hbm, hbm, vmem, hbm, hbm, hbm, hbm],
        out_specs=[hbm, hbm, hbm, vmem, hbm, hbm, hbm],
        out_shape=[sds((S, D), BF), sds((S, D), BF), sds((D, 3 * D), BF), sds((D, DH), BF),
                   sds((D, D), BF), sds((D, F), BF), sds((F, D), BF)],
        scratch_shapes=[
            V((S, D), BF), V((S, D), BF), V((D, D), BF),
            V((NC, D, FC), BF), V((NC, FC, D), BF),
            V((S, D), BF), V((NT, D, T), BF), V((NT, D, T), BF), V((D, 128), BF),
            V((3, NT, D, T), BF), V((NT, D, T), BF), V((NC, S, FC), BF), V((NT, D, T), BF),
            V((2 * G, 8, T), F32), V((4, HS, HD), F32),
            V((2 * G, PR + EXT, 128), F32), V((2 * G, PR + EXT, 128), BF), V((2 * G, 128, 128), BF),
            V((2 * G, 128, 128), F32), V((5, HS, HD), BF), V((5, NT, HD, TH), BF), V((5, HD, HD), BF),
            dma((2 * NT,)), dma((2 * NT,)), dma((6,)), dma((1,)), dma((NC,)), dma((NC,)),
            dma((2 * NT,)), dma((2 * NT,)), dma((6,)), dma((1,)), dma((NC,)), dma((NC,)),
        ],
        compiler_params=pltpu.CompilerParams(vmem_limit_bytes=128 * 1024 * 1024),
    )(A_x.reshape(S, D), A_wqkv, A_w_phi.reshape(D, DH), A_wo, B_w1, B_w2, grad_out.reshape(S, D))
    return (out.reshape(1, S, D), dx.reshape(1, S, D), dwqkv, dwphi.reshape(H, DH, DH), dwo, dw1, dw2)
```

```python
import jax
import jax.numpy as jnp
from jax import lax
import jax.experimental.pallas as pl
import jax.experimental.pallas.tpu as pltpu

S, D, H, F = 2048, 1024, 32, 3584
DH = D // H
T = 512
NT = S // T
FC = 512
NC = F // FC
G = D // 128
HS, HD, HF, TH, GH = S // 2, D // 2, FC // 2, T // 2, 3 * G // 2
PR = 2 * DH
RB = 32
EXT = 16
BF, F32 = jnp.bfloat16, jnp.float32


def _nn(a, b):
    return lax.dot_general(a, b, (((1,), (0,)), ((), ())), preferred_element_type=F32)


def _nt(a, b):
    return lax.dot_general(a, b, (((1,), (1,)), ((), ())), preferred_element_type=F32)


def _tn(a, b):
    return lax.dot_general(a, b, (((0,), (0,)), ((), ())), preferred_element_type=F32)


def _sums(q11, q12, q21, q22):
    a, b, c, d = (q.astype(F32) for q in (q11, q12, q21, q22))
    return [v.astype(BF) for v in (a + d, c + d, a + b, c - a, b - d)]


def _lazy(q):
    f = lambda k: q(k).astype(F32)
    return (lambda: q(0), lambda: q(3),
            [lambda: (f(0) + f(3)).astype(BF), lambda: (f(2) + f(3)).astype(BF), lambda: (f(0) + f(1)).astype(BF),
             lambda: (f(2) - f(0)).astype(BF), lambda: (f(1) - f(3)).astype(BF)])


def _as_lhs(q11, q22, s):
    return [s[0], s[1], q11, q22, s[2], s[3], s[4]]


def _as_rhs(q11, q22, s):
    return [s[0], q11, s[4], s[3], q22, s[2], s[1]]


_USES = ({0: 1, 3: 1}, {2: 1, 3: -1}, {1: 1, 3: 1}, {0: 1, 2: 1}, {0: -1, 1: 1}, {3: 1}, {0: 1})


def _strassen(dot, a, b, done=lambda k, v: v, fill=(), order=(1, 3, 4, 2, 0, 6, 5)):
    get = lambda v: v() if callable(v) else v
    c, left = {}, [4, 2, 2, 4]
    for n, i in enumerate(order):
        m = dot(get(a[i]), get(b[i]))
        if n < len(fill):
            fill[n]()
        for k, sign in _USES[i].items():
            if k not in c:
                c[k] = (sign, m)
            else:
                c[k] = (1, m - c[k][1] if c[k][0] < 0 else c[k][1] + m if sign > 0 else c[k][1] - m)
            left[k] -= 1
            if not left[k]:
                c[k] = done(k, c[k][1])
    return [c[k] for k in range(4)]


def _quads(v):
    nr, nc = v.shape[0] // 2, v.shape[1] // 2
    return [v[_half(k // 2, nr), _half(k % 2, nc)] for k in range(4)]


def _join(q):
    return jnp.concatenate([jnp.concatenate(q[:2], axis=1), jnp.concatenate(q[2:], axis=1)], axis=0)


def _level2(dot):
    def ops(v, flip):
        if isinstance(v, tuple):
            return v
        q = _quads(v)
        return q[0], q[3], _sums(q[0], q[1 + flip], q[2 - flip], q[3])

    return lambda a, b: _join(_strassen(dot, _as_lhs(*ops(a, 0)), _as_rhs(*ops(b, int(dot is _nt)))))


def _softmax_pm(p):
    p3 = p.reshape(-1, DH, p.shape[-1])
    ep = jnp.exp(p3 - jnp.max(p3, axis=1, keepdims=True))
    em = jnp.exp(jnp.min(p3, axis=1, keepdims=True) - p3)
    sp = ep * (1.0 / jnp.sum(ep, axis=1, keepdims=True))
    sm = em * (1.0 / jnp.sum(em, axis=1, keepdims=True))
    return sp.reshape(p.shape), sm.reshape(p.shape)


def _softmax_pm_bwd(php, phm, dp, dm):
    n = php.shape[-1]
    a, b = php.reshape(-1, DH, n), phm.reshape(-1, DH, n)
    ta, tb = a * dp.reshape(-1, DH, n), b * dm.reshape(-1, DH, n)
    r = (ta - tb) - a * jnp.sum(ta, axis=1, keepdims=True) + b * jnp.sum(tb, axis=1, keepdims=True)
    return r.reshape(php.shape)


def _finish_state(acc_ref, ext_ref, t_ref, col_ref):
    r = lax.broadcasted_iota(jnp.int32, (PR + EXT, 128), 0)
    c = lax.broadcasted_iota(jnp.int32, (PR + EXT, 128), 1)
    mask = jnp.where(r < PR, r // DH, r - PR) == (c % PR) // DH
    zero = jnp.zeros((PR, 128), F32)
    for p in range(2 * G):
        st = jnp.where(mask, acc_ref[p], 0.0).astype(BF)
        acc_ref[p] = jnp.zeros((PR + EXT, 128), F32)
        ext_ref[p] = st
        st = st.astype(F32)
        t_ref[p] = jnp.concatenate([st[:PR], zero][::1 - 2 * (p % 2)], axis=0).T.astype(BF)
        col_ref[p] = jnp.broadcast_to(jnp.sum(st[PR:], axis=0, keepdims=True), (128, 128)).T


def _pair(plus, minus, i):
    return jnp.concatenate([plus[_half(i, PR)], minus[_half(i, PR)]], axis=0)


def _lanes(col):
    return jnp.concatenate([col] * (T // 128), axis=1)


def _normalize(x):
    x = x.astype(F32)
    xc = x - jnp.mean(x, axis=1, keepdims=True)
    rstd = lax.rsqrt(jnp.mean(xc * xc, axis=1, keepdims=True) + 1e-5)
    return xc * rstd, rstd


def _half(i, n):
    return slice(i * n, (i + 1) * n)


def _kernel(x_hbm, wqkv_hbm, wphi_hbm, wo_hbm, w1_hbm, w2_hbm, go_hbm,
            out_hbm, dx_hbm, dwqkv_hbm, dwphi_hbm, dwo_hbm, dw1_hbm, dw2_hbm,
            x_v, go_v, wo_v, w1_v, w2_v, xn_v, wT_v, bd_v,
            qkvT_v, pkm_v, h_v, oT_v, rd_v, m_v, acc_v, ext_v, stT_v, col_v, ts_v, fs_v, fs2_v, wos_v, wphi_v,
            sem_x, sem_go, sem_wqkv, sem_wo, sem_w1, sem_w2,
            sem_out, sem_dx, sem_dwqkv, sem_dwo, sem_dw1, sem_dw2):
    cp = pltpu.make_async_copy

    def rows(t, j):
        return pl.ds(pl.multiple_of(j * HS + t * TH, TH), TH)

    def qrows(t):
        return pl.ds(pl.multiple_of(t * TH, TH), TH)

    def tile_cp(src, dst, sem, t):
        return [cp(src.at[rows(t, j), :], dst.at[rows(t, j), :], sem.at[2 * t + j]) for j in range(2)]

    def start(cs):
        for c in cs:
            c.start()

    def wait(cs):
        for c in cs:
            c.wait()

    def fquad(ref, i, j):
        return jnp.concatenate([ref[t, _half(i, HD), _half(j, TH)] for t in range(NT)], axis=1)

    def xnT_lhs():
        cat = lambda f: lambda: jnp.concatenate([f(t) for t in range(NT)], axis=1)
        ops = [(cat(lambda t, k=k: fs_v[k, t, :HF, :128]), cat(lambda t, k=k: fs_v[k, t, HF:, 128:]),
                [cat(lambda t, k=k, j=j: fs2_v[k, j, t]) for j in range(5)]) for k in range(7)]
        return _as_lhs(ops[5], ops[6], ops)

    by_half = [2 * t + p for p in range(2) for t in range(NT)]

    x_in = lambda t: tile_cp(x_hbm, x_v, sem_x, t)
    go_in = lambda t: tile_cp(go_hbm, go_v, sem_go, t)
    out_out = lambda t: tile_cp(x_v, out_hbm, sem_out, t)
    dx_out = lambda t: tile_cp(xn_v, dx_hbm, sem_dx, t)

    def wqkv_in(k):
        return cp(wqkv_hbm.at[:, fcols(k)], qkvT_v.at[k // 2, k % 2], sem_wqkv.at[k])

    def wqkv_again(k):
        return cp(wqkv_hbm.at[:, fcols(k)], w1_v.at[k], sem_wqkv.at[k])

    def fcols(c):
        return pl.ds(pl.multiple_of(c * FC, FC), FC)

    def w_in(c):
        return [cp(w1_hbm.at[:, fcols(c)], w1_v.at[c], sem_w1.at[c]),
                cp(w2_hbm.at[fcols(c), :], w2_v.at[c], sem_w2.at[c])]

    def dw1_out(c):
        return cp(h_v.at[c, :D, :], dw1_hbm.at[:, fcols(c)], sem_dw1.at[c])

    def dw2_out(c):
        return cp(w2_v.at[c], dw2_hbm.at[fcols(c), :], sem_dw2.at[c])

    def dwqkv_out(k):
        return cp(wT_v.at[k], dwqkv_hbm.at[:, fcols(k)], sem_dwqkv.at[k])

    def dwv_out(j):
        return cp(pkm_v.at[j], dwqkv_hbm.at[:, fcols(4 + j)], sem_dwqkv.at[4 + j])

    wo_in = cp(wo_hbm, wo_v, sem_wo.at[0])
    wphi_in = cp(wphi_hbm, wphi_v, sem_wo.at[1])
    dwphi_out = cp(wphi_v, dwphi_hbm, sem_wo.at[1])
    dwo_out = [cp(wos_v.at[k], dwo_hbm.at[_half(k // 2, HD), _half(k % 2, HD)], sem_dwo.at[k]) for k in range(4)]
    go_again = [cp(go_hbm.at[_half(k // 2, HS), _half(k % 2, HD)], ts_v.at[k], sem_go.at[k]) for k in range(4)]

    start(x_in(0))

    def zero_body(k, carry):
        m_v[k] = jnp.zeros((HS, HD), F32)
        return carry

    lax.fori_loop(0, 4, zero_body, 0)

    def ln_body(t, carry):
        wait(x_in(t))
        pl.when(t < NT - 1)(lambda: start(x_in(t + 1)))
        pl.when(t == NT - 2)(lambda: start(w_in(0)))
        xn = [_normalize(x_v[rows(t, j), :])[0] for j in range(2)]
        for j in range(2):
            xn_v[rows(t, j), :] = xn[j].astype(BF)
        for k, u in enumerate(_sums(*[xn[k // 2][:, _half(k % 2, HD)] for k in range(4)])):
            ts_v[k, qrows(t), :] = u
        for g in range(2):
            ops = []
            for r in (g, g + 2):
                q = [xn_v[rows(t, k % 2), _half(4 * (k // 2) + r, 128)].T for k in range(4)]
                ops.append(_sums(*q) + [q[0], q[3]])
                for k in range(7):
                    fs_v[k, t, _half(r, 128), :] = ops[-1][k]
            for k in range(7):
                for j, u in enumerate(_sums(*[ops[i // 2][k][:, _half(i % 2, 128)] for i in range(4)])):
                    fs2_v[k, j, t, _half(g, 128), :] = u
        return carry

    lax.fori_loop(0, NT, ln_body, 0)

    def quads(ref, c, nr, nc):
        return [ref[c, _half(k // 2, nr), _half(k % 2, nc)] for k in range(4)]

    def tok_ops(side):
        return side(lambda: xn_v[:HS, :HD], lambda: xn_v[HS:, HD:], [lambda k=k: ts_v[k] for k in range(5)])

    def add_m(k, v):
        m_v[k] += v

    def put(ref, nr, nc):
        def store(k, v):
            ref[_half(k // 2, nr), _half(k % 2, nc)] = v.astype(BF)
        return store

    tall = lambda ref: [ref.at[k // 2, :, _half(k % 2, HF)] for k in range(7)]

    def ff_body(c, carry):
        wait(w_in(c))

        @pl.when(c < NC - 1)
        def _():
            start(w_in(c + 1))
            wqkv_in(c).start()

        w = quads(w1_v, c, HD, HF)

        def act(k, h):
            h = h.astype(BF)
            h_v[c, _half(k // 2, HS), _half(k % 2, HF)] = h
            tall(oT_v)[k][...] = jnp.maximum(h, 0)

        _strassen(_nn, tok_ops(_as_lhs), _as_rhs(w[0], w[3], _sums(*w)), act)
        w = quads(w2_v, c, HF, HD)
        _strassen(_nn, _as_lhs(*_lazy(lambda k: tall(oT_v)[k][...])), _as_rhs(w[0], w[3], _sums(*w)), add_m,
                  order=(2, 4, 5, 3, 1, 0, 6))
        return carry

    wphi_in.start()
    wo_in.start()
    lax.fori_loop(0, NC, ff_body, 0)
    wphi_in.wait()

    r = lax.broadcasted_iota(jnp.int32, (DH, 128), 0)
    c_ = lax.broadcasted_iota(jnp.int32, (DH, 128), 1)
    rep = _nn(wphi_v[...], (r == c_ % DH).astype(BF))
    r = lax.broadcasted_iota(jnp.int32, (D, 128), 0)
    c_ = lax.broadcasted_iota(jnp.int32, (D, 128), 1)
    bd_v[...] = jnp.where((r % 128) // DH == c_ // DH, rep, 0.0).astype(BF)

    acc_v[...] = jnp.zeros(acc_v.shape, F32)
    slots = ([ts_v.at[k // 2, _half(k % 2, HD), :] for k in range(10)]
             + [oT_v.at[k // 2, _half(k % 2, HD), :] for k in range(8)]
             + [xn_v.at[_half(k, HD), :HD] for k in range(3)])

    def w_rows(g):
        w = qkvT_v[g // G, g % G // 4, :, _half(g % 4, 128)]
        return w.T if g // G == 2 else _nt(bd_v[_half(g % G, 128), :].T, w)

    for k in range(6):
        wqkv_in(k).wait()
    wo_in.wait()
    for t in range(NT):
        start(go_in(t))
    for k, u in enumerate(_sums(wo_v[:HD, :HD], wo_v[:HD, HD:], wo_v[HD:, :HD], wo_v[HD:, HD:])):
        wos_v[k] = u
    for g in (0, 4, 8, 1, 5, 9, 2, 6, 10, 3, 7, 11):
        top, bot = w_rows(g // 4 * G + g % 4), w_rows(g // 4 * G + g % 4 + 4)
        for p in range(4):
            q = [v[_half(p, 32), _half(i, HD)] for v in (top, bot) for i in range(2)]
            for k, u in enumerate(_as_lhs(q[0].astype(BF), q[3].astype(BF), _sums(*q))):
                slots[3 * k + g // 4][_half(4 * (g % 4) + p, 32), :] = u


    def p1_body(t, carry):
        q = _strassen(_nn, [lambda k=k: jnp.concatenate([v[...] for v in slots[3 * k:3 * k + 3]], axis=0) for k in range(7)],
                      _as_rhs(fs_v[5, t], fs_v[6, t], [fs_v[k, t] for k in range(5)]))

        def proj(g):
            rs, hi = _half(g // G * 4 + g % 4, 128), g % G // 4
            return jnp.concatenate([q[2 * hi][rs], q[2 * hi + 1][rs]], axis=1)

        ones = jnp.ones((EXT, T), BF)
        for g in (4, 5, 6, 7, 0, 1, 2, 3):
            gs = _half(g, 128)
            sp, sm = _softmax_pm(proj(g))
            qkvT_v[0, t, gs, :] = sp.astype(BF)
            wT_v[t, gs, :] = sm.astype(BF)
            sp, sm = _softmax_pm(proj(G + g))
            sp, sm = sp.astype(BF), sm.astype(BF)
            v = proj(2 * G + g).astype(BF)
            qkvT_v[1, t, gs, :] = sp
            pkm_v[t, gs, :] = sm
            qkvT_v[2, t, gs, :] = v
            for i in range(2):
                acc_v[2 * g + i] += _nt(jnp.concatenate([v[_half(i, PR)], ones], axis=0), _pair(sp, sm, i))
        return carry

    lax.fori_loop(0, NT, p1_body, 0)
    _finish_state(acc_v, ext_v, stT_v, col_v)

    def head_rows(v):
        return jnp.concatenate([jnp.broadcast_to(v[j:j + 1], (DH, T)) for j in range(2)], axis=0)

    def phi_q(t, p):
        return jnp.concatenate([qkvT_v[0, t, _half(p, PR), :], wT_v[t, _half(p, PR), :]], axis=0)

    def state_T(g):
        return jnp.concatenate([stT_v[2 * g], stT_v[2 * g + 1]], axis=0)

    def p2_body(t, carry):
        wait(go_in(t))
        o_tok, gate, dgate, ds = [], {}, {}, {}
        for g in range(G):
            gs = _half(g, 128)
            o = []
            for p in (2 * g, 2 * g + 1):
                nd = _nn(ext_v[p], phi_q(t, p))
                rd = 1.0 / (nd[PR:PR + 8] + 1e-6)
                rd_v[p] = rd
                o.append(nd[:PR] * head_rows(rd))
            o = jnp.concatenate(o, axis=0)
            oT_v[t, gs, :] = o.astype(BF)
            o_tok.append(o.astype(BF).T)
            k, cs = g // 2, _half(g % 2, HD // 2)
            at = (rows(t, k // 2), _half(2 * (k % 2) + g % 2, HD // 2))
            m = m_v[k, qrows(t), cs]
            sig = 1.0 / (1.0 + jnp.exp(-m))
            go = go_v[at].astype(F32)
            gate[g] = m * sig
            dgate[g] = go * (sig + gate[g] * (1.0 - sig))
            ds[g] = (go * gate[g]).astype(BF)
            go_v[at] = ds[g]
        gate, dgate, ds = ([jnp.concatenate([v[2 * k], v[2 * k + 1]], axis=1) for k in range(4)]
                           for v in (gate, dgate, ds))
        wo = (lambda: wo_v[:HD, :HD], lambda: wo_v[HD:, HD:], [lambda k=k: wos_v[k] for k in range(5)])
        do = _strassen(_nt, _as_lhs(*wo), _as_rhs(ds[0], ds[3], _sums(ds[0], ds[2], ds[1], ds[3])))
        sub = lax.broadcasted_iota(jnp.int32, (EXT, T), 0)

        def group_bwd(g):
            gs = _half(g, 128)
            dnum = jnp.concatenate([v[_half(g % 4, 128)] for v in do[_half(g // 4, 2)]], axis=1)
            dnum = dnum * jnp.concatenate([head_rows(rd_v[2 * g]), head_rows(rd_v[2 * g + 1])], axis=0)
            tt = dnum * oT_v[t, gs, :].astype(F32)
            dnum = dnum.astype(BF)
            dphis = _nn(state_T(g), dnum)
            for i in range(2):
                p = 2 * g + i
                dd = [-jnp.sum(tt[_half(2 * i + j, DH)], axis=0, keepdims=True) for j in range(2)]
                dden_ext = jnp.where(sub == 0, jnp.broadcast_to(dd[0], (EXT, T)), jnp.broadcast_to(dd[1], (EXT, T)))
                dden = jnp.concatenate([jnp.broadcast_to(dd[j % 2], (DH, T)) for j in range(4)], axis=0)
                phi = phi_q(t, p)
                acc_v[p] += _nt(jnp.concatenate([dnum[_half(i, PR)], dden_ext.astype(BF)], axis=0), phi)
                dphi = dphis[_half(i, 128)] + _lanes(col_v[p]) * dden
                phi = phi.astype(F32)
                qkvT_v[0, t, _half(p, PR), :] = _softmax_pm_bwd(phi[:PR], phi[PR:], dphi[:PR], dphi[PR:]).astype(BF)

        def gated(k, s):
            at = (rows(t, k // 2), _half(k % 2, HD))
            x_v[at] = (x_v[at].astype(F32) + s * gate[k]).astype(BF)
            dm = (s * dgate[k]).astype(BF)
            xn_v[at] = dm
            m_v[k, qrows(t), :] = jnp.zeros((TH, HD), F32)
            return dm

        o = [jnp.concatenate([v[_half(k // 2, TH)] for v in o_tok[_half(k % 2, 4)]], axis=1) for k in range(4)]
        o = _as_lhs(o[0], o[3], _sums(*o))
        group_bwd(0)
        group_bwd(1)
        dm = _strassen(_nn, o, _as_rhs(*wo), gated, [lambda g=g: group_bwd(g) for g in range(2, G)])
        for k, u in enumerate(_sums(*dm)):
            ts_v[k, qrows(t), :] = u
        start(out_out(t))
        return carry

    lax.fori_loop(0, NT, p2_body, 0)

    _finish_state(acc_v, ext_v, stT_v, col_v)

    dm_ops = [ts_v.at[k] for k in range(5)] + [xn_v.at[:HS, :HD], xn_v.at[HS:, HD:]]
    dm_slots = ([ts_v.at[0, :HD, HF:]] + [wos_v.at[k // 2, :, _half(k % 2, HF)] for k in range(10)]
                + [xn_v.at[_half(k // 2, HD), _half(k % 2 + 2 * (k < 4), HF)] for k in range(8)]
                + [x_v.at[_half(k // 4, HD), _half(k % 4, HF)] for k in range(16)])

    def dm_split(r, carry):
        r0 = pl.multiple_of(r * PR, PR)
        for k, v in enumerate(dm_ops):
            for j, u in enumerate(_sums(*[v[pl.ds(i // 2 * HD + r0, PR), _half(i % 2, HF)] for i in range(4)])):
                dm_slots[5 * k + j][pl.ds(r0, PR), :] = u
        return carry

    def dm2(side):
        ops = [(lambda v=v: v[:HD, :HF], lambda v=v: v[HD:, HF:], [lambda u=u: u[...] for u in dm_slots[5 * k:5 * k + 5]])
               for k, v in enumerate(dm_ops)]
        return side(ops[5], ops[6], ops)

    for t in range(NT):
        wait(out_out(t))
    lax.fori_loop(0, HD // PR, dm_split, 0)

    def pa_body(c, carry):
        def act_bwd(k, da, p):
            at = (c, _half(2 * (k // 2) + p, HD), _half(k % 2, HF))
            h = h_v[at].astype(F32)
            h_v[at] = (da[_half(p, HD)] * jnp.where(h > 0, 1.0, jnp.where(h == 0, 0.5, 0.0))).astype(BF)

        def flip(k):
            v = jnp.maximum(h_v[c, _half(k % 2, HS), _half(k // 2, HF)].T, 0)
            for p in range(2):
                wT_v[k, _half(p, HF), :] = v[:, _half(p, HD)]

        aT = _lazy(lambda k: jnp.concatenate([wT_v[k, _half(p, HF), :] for p in range(2)], axis=1))
        w = quads(w2_v, c, HF, HD)
        da = _strassen(_level2(_nt), dm2(_as_lhs), _as_rhs(w[0], w[3], _sums(w[0], w[2], w[1], w[3])),
                       fill=[lambda k=k: flip(k) for k in range(4)])
        _strassen(_level2(_nn), _as_lhs(*aT), dm2(_as_rhs),
                  put(w2_v.at[c], HF, HD),
                  [lambda k=k: [act_bwd(k, da[k], p) for p in range(2)] for k in (2, 1, 0, 3)], order=(2, 4, 5, 3, 1, 0, 6))
        dw2_out(c).start()
        return carry

    lax.fori_loop(0, NC, pa_body, 0)

    for t in range(NT):
        start(x_in(t))
    start(go_again)

    def pb_body(c, carry):
        q11, q22, sums = _lazy(lambda k: h_v[c, _half(k // 2, HS), _half(k % 2, HF)])
        sums.append(q11)
        views = tall(wT_v)

        def keep(k):
            views[k][...] = sums[k]()

        dh = (lambda: views[5][...], q22, [lambda v=v: v[...] for v in views])
        keep(1)
        w = quads(w1_v, c, HD, HF)
        _strassen(_nt, _as_lhs(*dh), _as_rhs(w[0], w[3], _sums(w[0], w[2], w[1], w[3])), add_m,
                  [lambda k=k: keep(k) for k in (2, 5, 0, 4, 3)])
        regroup = lambda f: lambda: jnp.concatenate([f()[_half(b, 128)] for b in by_half], axis=0)
        _strassen(_level2(_nn), xnT_lhs(), [regroup(f) for f in _as_rhs(*dh)], put(h_v.at[c], HD, HF))
        dw1_out(c).start()
        return carry

    lax.fori_loop(0, NC, pb_body, 0)

    for k in range(6):
        wqkv_again(k).start()
    def p4_body(t, carry):
        for g in range(G):
            gs = _half(g, 128)
            dphis = _nn(state_T(g), qkvT_v[2, t, gs, :])
            for i in range(2):
                p = 2 * g + i
                ps = _half(p, PR)
                php, phm = qkvT_v[1, t, ps, :], pkm_v[t, ps, :]
                dv = _nn(ext_v[p, :PR, :], jnp.concatenate([php, phm], axis=0))
                dphi = dphis[_half(i, 128)] + _lanes(col_v[p])
                dpk = _softmax_pm_bwd(php.astype(F32), phm.astype(F32), dphi[:PR], dphi[PR:])
                qkvT_v[1, t, ps, :] = dpk.astype(BF)
                qkvT_v[2, t, ps, :] = dv.astype(BF)
        return carry

    lax.fori_loop(0, NT, p4_body, 0)

    def proj_grad(i):
        b = _lazy(lambda k: jnp.concatenate(
            [qkvT_v[i, u // 2, _half(k % 2, HD), _half(2 * (k // 2) + u % 2, 128)] for u in by_half], axis=1))
        q = _strassen(_level2(_nt), xnT_lhs(), _as_rhs(*b), lambda k, v: v.astype(BF))
        return [jnp.concatenate([q[j], q[2 + j]], axis=0) for j in range(2)]

    def put_w(i, w):
        ops = _as_lhs(w[0][:HD].astype(BF), w[1][HD:].astype(BF), _sums(w[0][:HD], w[1][:HD], w[0][HD:], w[1][HD:]))
        for k in range(7):
            h_v[k, pl.ds(pl.multiple_of(i * HD, HD), HD), :] = ops[k]

    col_v[:G] = jnp.zeros((G, 128, 128), F32)

    def p5_body(i, carry):
        for j in range(2):
            wqkv_again(2 * i + j).wait()
        gi = proj_grad(i)
        for j in range(2):
            pkm_v[j] = gi[j]

        @pl.when(i < 2)
        def _():
            folded = []
            for g in range(G):
                gs, ls = _half(g, 128), _half(g % 4, 128)
                bd, w, gg = bd_v[gs, :], w1_v[2 * i + g // 4, :, ls], pkm_v[g // 4, :, ls]
                wT_v[2 * i + g // 4, :, ls] = _nt(gg, bd).astype(BF)
                col_v[g] += _tn(w, gg)
                folded.append(_nn(w, bd))
            put_w(i, [jnp.concatenate(folded[:4], axis=1), jnp.concatenate(folded[4:], axis=1)])
            for j in range(2):
                dwqkv_out(2 * i + j).start()

        return carry

    for c in range(NC):
        dw1_out(c).wait()
    lax.fori_loop(0, 3, p5_body, 0)
    for j in range(2):
        dwv_out(j).start()
    put_w(2, [w1_v[4], w1_v[5]])
    for g in range(G):
        for j in range(4):
            hs = _half(j, DH)
            wphi_v[_half(4 * g + j, DH), :] = col_v[g, hs, :][:, hs].astype(BF)

    def ln_bwd(t, j, p):
        for e in range(128 // RB):
            r0 = pl.multiple_of(t * TH + p * 128 + e * RB, RB)
            at = pl.ds(pl.multiple_of(j * HS + r0, RB), RB)
            d = jnp.concatenate([m_v[2 * j + i, pl.ds(r0, RB), :] for i in range(2)], axis=1)
            xn, rstd = _normalize(x_v[at, :])
            m1 = jnp.mean(d, axis=1, keepdims=True)
            m2 = jnp.mean(d * xn, axis=1, keepdims=True)
            go = jnp.concatenate([ts_v[2 * j + i, pl.ds(r0, RB), :] for i in range(2)], axis=1)
            xn_v[at, :] = (go.astype(F32) + (d - m1 - xn * m2) * rstd).astype(BF)

    def p6_body(t, carry):
        b = _lazy(lambda k: jnp.concatenate(
            [qkvT_v[i, t, _half(k // 2, HD), _half(k % 2, TH)] for i in range(3)], axis=0))
        a = [lambda k=k: jnp.concatenate([h_v[k, _half(i, HD), :] for i in range(3)], axis=1) for k in range(7)]

        prev = lambda j, p: lambda: ln_bwd(jnp.maximum(t - 1, 0), j, p)

        def finish(k, v):
            m_v[2 * (k % 2) + k // 2, qrows(t), :] += v.astype(BF).T.astype(F32)

        _strassen(_nn, a, _as_rhs(*b), finish,
                  [lambda: None, prev(0, 0), prev(0, 1), prev(1, 0), prev(1, 1)])

        @pl.when(t > 0)
        def _():
            start(dx_out(t - 1))

        return carry

    for t in range(NT):
        wait(x_in(t))
    wait(go_again)
    dwphi_out.start()
    lax.fori_loop(0, NT, p6_body, 0)

    def last(j):
        for p in range(2):
            ln_bwd(NT - 1, j, p)

    def send(k, v):
        wos_v[k] = v.astype(BF)
        dwo_out[k].start()

    o = _lazy(lambda k: fquad(oT_v, k // 2, k % 2))
    d = _lazy(lambda k: go_v[_half(k // 2, HS), _half(k % 2, HD)])
    _strassen(_nn, _as_lhs(*o), _as_rhs(*d), send,
              [lambda: last(0), lambda: None, lambda: last(1), lambda: start(dx_out(NT - 1))])

    for c in range(NC):
        dw2_out(c).wait()
    wait(dwo_out)
    dwphi_out.wait()
    for k in range(4):
        dwqkv_out(k).wait()
    for j in range(2):
        dwv_out(j).wait()
    for t in range(NT):
        wait(dx_out(t))


@jax.jit
def pallas_recurrent_scan__linear_kernel_hedgehog__dense_activation_relu__prompt_kernel(
    A_x: jax.Array,
    A_wqkv: jax.Array,
    A_w_phi: jax.Array,
    A_wo: jax.Array,
    B_x: jax.Array,
    B_w1: jax.Array,
    B_w2: jax.Array,
    grad_out: jax.Array,
):
    del B_x
    hbm = pl.BlockSpec(memory_space=pl.ANY)
    sds = jax.ShapeDtypeStruct
    V = pltpu.VMEM
    dma = pltpu.SemaphoreType.DMA
    out, dx, dwqkv, dwphi, dwo, dw1, dw2 = pl.pallas_call(
        _kernel,
        in_specs=[hbm, hbm, hbm, hbm, hbm, hbm, hbm],
        out_specs=[hbm, hbm, hbm, hbm, hbm, hbm, hbm],
        out_shape=[sds((S, D), BF), sds((S, D), BF), sds((D, 3 * D), BF), sds((D, DH), BF),
                   sds((D, D), BF), sds((D, F), BF), sds((F, D), BF)],
        scratch_shapes=[
            V((S, D), BF), V((S, D), BF), V((D, D), BF),
            V((NC, D, FC), BF), V((NC, FC, D), BF),
            V((S, D), BF), V((NT, D, T), BF), V((D, 128), BF),
            V((3, NT, D, T), BF), V((NT, D, T), BF), V((NC, S, FC), BF), V((NT, D, T), BF),
            V((2 * G, 8, T), F32), V((4, HS, HD), F32),
            V((2 * G, PR + EXT, 128), F32), V((2 * G, PR + EXT, 128), BF), V((2 * G, 128, 128), BF),
            V((2 * G, 128, 128), F32), V((5, HS, HD), BF), V((7, NT, HD, TH), BF), V((7, 5, NT, HF, 128), BF), V((5, HD, HD), BF), V((D, DH), BF),
            dma((2 * NT,)), dma((2 * NT,)), dma((6,)), dma((4,)), dma((NC,)), dma((NC,)),
            dma((2 * NT,)), dma((2 * NT,)), dma((6,)), dma((4,)), dma((NC,)), dma((NC,)),
        ],
        compiler_params=pltpu.CompilerParams(vmem_limit_bytes=128 * 1024 * 1024),
    )(A_x.reshape(S, D), A_wqkv, A_w_phi.reshape(D, DH), A_wo, B_w1, B_w2, grad_out.reshape(S, D))
    return (out.reshape(1, S, D), dx.reshape(1, S, D), dwqkv, dwphi.reshape(H, DH, DH), dwo, dw1, dw2)
```
